```python
import os as _os
_os.environ.setdefault("JAX_PLATFORMS", "cpu")
import jax
import jax.numpy as jnp

def _softmax(x, axis=-1):
    return jax.nn.softmax(x, axis=axis)
def _gelu(x):
    return jax.nn.gelu(x, approximate=True)
def _silu(x):
    return jax.nn.silu(x)
def _sigmoid(x):
    return jax.nn.sigmoid(x)
def _layernorm(x, axis=-1, eps=1e-5):
    m = jnp.mean(x, axis=axis, keepdims=True)
    v = jnp.var(x, axis=axis, keepdims=True)
    return (x - m) / jnp.sqrt(v + eps)
def _scatter_add(tgt, idx, src, axis=0):
    return tgt.at[idx].add(src)
def _segment_sum(src, seg, n):
    return jax.ops.segment_sum(src, seg, n)
class _Rng:
    def __init__(self, key):
        self._k = key
    def _next(self):
        self._k, sub = jax.random.split(self._k)
        return sub
    def normal(self, shape):
        return jax.random.normal(self._next(), shape, dtype=jnp.bfloat16)
    def randint(self, lo, hi, shape):
        return jax.random.randint(self._next(), shape, lo, hi, dtype=jnp.int32)
    def uniform(self, shape, lo=0.0, hi=1.0):
        return jax.random.uniform(self._next(), shape, jnp.bfloat16, lo, hi)
    def permutation(self, n):
        return jax.random.permutation(self._next(), n)


kernel_name = 'concat_heads__grouped_kv_mqa__sliding_block__prompt'

def setup_inputs():
    _rng = _Rng(jax.random.key(int.from_bytes(__import__("os").urandom(4), "little")))
    _w = (lambda a: (lambda t: t.astype(jnp.bfloat16) if jnp.issubdtype(t.dtype, jnp.floating) else t)(jnp.asarray(a)))
    def _A_setup():
        B, S, D, H = 1, 2048, 1024, 32
        Dh = D // H
        return {
            "x": _w((lambda *s: _rng.normal(s) * 0.05)(B, S, D)),
            "wq": _w((lambda *s: _rng.normal(s) * 1.6)(D, H * Dh)),
            "wk": _w((lambda *s: _rng.normal(s) * 1.6)(D, Dh)),
            "wv": _w((lambda *s: _rng.normal(s) * 0.1)(D, Dh)),
            "wo": _w((lambda *s: _rng.normal(s) * 0.1)(H * Dh, D)),
        }
    _A_in = _A_setup()

    def _B_setup():
        B, S, D = 1, 2048, 1024
        return {
            "x": _w((lambda *s: _rng.normal(s) * 0.2)(B, S, D)),
            "wqkv": _w((lambda *s: _rng.normal(s) * 0.2)(D, 3 * D)),
            "wo": _w((lambda *s: _rng.normal(s) * 0.05)(D, D)),
        }
    _B_in = _B_setup()

    return {
        "A_x": _A_in["x"],
        "A_wq": _A_in["wq"],
        "A_wk": _A_in["wk"],
        "A_wv": _A_in["wv"],
        "A_wo": _A_in["wo"],
        "B_x": _B_in["x"],
        "B_wqkv": _B_in["wqkv"],
        "B_wo": _B_in["wo"],
    }

def reference(A_x, A_wq, A_wk, A_wv, A_wo, B_x, B_wqkv, B_wo):
    def _A_ref(x, wq, wk, wv, wo):
        B, S, D = x.shape
        H = 32
        Dh = D // H
        q = (lambda x, *d: x.transpose(*d))((x @ wq).reshape(B, S, H, Dh), 0, 2, 1, 3)
        k = x @ wk
        v = x @ wv
        scores = jnp.einsum("bhqd,bkd->bhqk", q, k) * (Dh ** -0.5)
        p = _softmax(scores, axis=-1)
        o = jnp.einsum("bhqk,bkd->bhqd", p, v)
        return (lambda x, *d: x.transpose(*d))(o, 0, 2, 1, 3).reshape(B, S, H * Dh) @ wo

    def _B_ref(x, wqkv, wo):
        B, S, D = x.shape
        H = 32; Dh = D // H; W = 256
        qkv = (lambda x, *d: x.transpose(*d))((x @ wqkv).reshape(B, S, 3, H, Dh), 2, 0, 3, 1, 4)
        q, k, v = qkv[0], qkv[1], qkv[2]
        scores = jnp.einsum("bhqd,bhkd->bhqk", q, k) * (Dh ** -0.5)
        idx = jnp.arange(S)
        mask = (idx[:, None] - idx[None, :] >= 0) & (idx[:, None] - idx[None, :] < W)
        scores = jnp.where(mask[None, None], scores, -1e9)
        p = _softmax(scores, axis=-1)
        o = jnp.einsum("bhqk,bhkd->bhqd", p, v)
        return (lambda x, *d: x.transpose(*d))(o, 0, 2, 1, 3).reshape(B, S, D) @ wo

    a = _A_ref(A_x, A_wq, A_wk, A_wv, A_wo)
    b = _B_ref(B_x, B_wqkv, B_wo)
    return jnp.concatenate([a, b], axis=-1)
```

```python
import functools
import jax
import jax.numpy as jnp
from jax import lax
import jax.experimental.pallas as pl
import jax.experimental.pallas.tpu as pltpu

S = 2048
D = 1024
H = 32
DH = 32
NG = 8
TQ = 128
NT_ = S // TQ
PROFILE = False
LOG2E = 1.4426950408889634
QSCALE = (DH ** -0.5) * LOG2E
NEG = -1e30
BF = jnp.bfloat16
F32 = jnp.float32

_NN = (((1,), (0,)), ((), ()))
_NT = (((1,), (1,)), ((), ()))


def _dot(a, b):
    return lax.dot_general(a, b, _NN, preferred_element_type=F32)


def _dot_nt(a, b):
    return lax.dot_general(a, b, _NT, preferred_element_type=F32)


def _ds(i, n=128):
    if isinstance(i, int):
        return pl.ds(i * n, n)
    return pl.ds(pl.multiple_of(i * n, n), n)


def _chain(op, acc, x):
    for r in range(x.shape[0] // 8):
        sl = x[r * 8:(r + 1) * 8, :]
        acc = sl if acc is None else op(acc, sl)
    return acc


def _kernel(xa_h, wq_h, wk_h, wv_h, woa_h, xb_h, wqkv_h, wob_h, out_h,
            xa, wq, woa, xb, wqkv, wob,
            wta, wtb, qta, kpa, vta, oa, qtb, kb, vtb, ob,
            sa, sb, bias, acc_ref, l_ref, outa, outb,
            sem_x, sem_w, sem_o, *, NB, MB0, TC0, wait_all, STAGES, merge_a, merge_b, OA_CH, OB_CH, TCB):
    def cp(src, dst, sem):
        return pltpu.make_async_copy(src, dst, sem)

    _sc = [None]
    def scope(name):
        if not PROFILE:
            return
        if _sc[0] is not None:
            _sc[0].__exit__(None, None, None)
            _sc[0] = None
        if name is not None:
            _sc[0] = jax.named_scope(name)
            _sc[0].__enter__()
    scope('issue')
    a_chunks = [(0, TC0)]
    while a_chunks[-1][0] + a_chunks[-1][1] < S:
        s0 = a_chunks[-1][0] + a_chunks[-1][1]
        a_chunks.append((s0, min(512, S - s0)))
    xa_cp = [cp(xa_h.at[pl.ds(s0, n)], xa.at[pl.ds(s0, n)], sem_x.at[c]) for c, (s0, n) in enumerate(a_chunks)]
    wblocks = []
    m0 = 0
    for n in MB0:
        wblocks.append((m0, n))
        m0 += n
    assert m0 == D
    wq_cp = [cp(wq_h.at[:, pl.ds(m0, n)], wq.at[:, pl.ds(m0, n)], sem_w.at[j]) for j, (m0, n) in enumerate(wblocks)]
    wk_cp = cp(wk_h, wta.at[pl.ds(D, DH)], sem_w.at[8])
    wv_cp = cp(wv_h, wta.at[pl.ds(D + DH, DH)], sem_w.at[9])
    wqkv_cp = cp(wqkv_h, wqkv, sem_w.at[10])
    xb_cp = cp(xb_h, xb, sem_w.at[11])
    woa_cp = cp(woa_h, woa, sem_w.at[12])
    wob_cp = cp(wob_h, wob, sem_w.at[13])

    named = {'x%d' % c: d for c, d in enumerate(xa_cp)}
    named.update({'w%d' % j: d for j, d in enumerate(wq_cp)})
    named.update(wk=wk_cp, wv=wv_cp)

    def start_stage(k):
        if k < len(STAGES):
            for nm in STAGES[k]:
                if isinstance(nm, tuple):
                    named[nm[0]].start(priority=nm[1])
                else:
                    named[nm].start()

    start_stage(0)

    def kv_store(r, s0, n):
        cols = pl.ds(s0, n)
        kt = r[0:DH, :].astype(BF)
        vta[:, cols] = r[DH:2 * DH, :].astype(BF)
        kpa[cols, :] = jnp.concatenate([kt, jnp.zeros((128 - DH, n), BF)], axis=0).T

    s0, n = a_chunks[0]
    scope('w_x0')
    xa_cp[0].wait()
    for j, (m0, mn) in enumerate(wblocks):
        scope('w_w%d' % j)
        wq_cp[j].wait()
        start_stage(j + 1)
        scope('blk%d' % j)
        rows = pl.ds(m0, mn)
        for q in range(mn // 128):
            wta[pl.ds(m0 + q * 128, 128), :] = wq[:, pl.ds(m0 + q * 128, 128)].T
        if j < len(wblocks) - 1:
            qta[rows, pl.ds(s0, n)] = (_dot_nt(wta[rows, :], xa[pl.ds(s0, n), :]) * QSCALE).astype(BF)
        else:
            wk_cp.wait()
            wv_cp.wait()
            r = _dot_nt(wta[pl.ds(m0, mn + 2 * DH), :], xa[pl.ds(s0, n), :])
            qta[rows, pl.ds(s0, n)] = (r[0:mn, :] * QSCALE).astype(BF)
            kv_store(r[mn:mn + 2 * DH, :], s0, n)
    scope('w_xrest')
    start_stage(len(wblocks) + 1)
    if wait_all:
        for c in xa_cp[1:]:
            c.wait()

    def wtb_piece(j):
        src = j * 128 if j < 8 else 2 * D + (j - 8) * 128
        wtb[pl.ds(j * 128, 128), :] = wqkv[:, pl.ds(src, 128)].T

    scope('p0_rest')
    for c, (s0, n) in enumerate(a_chunks):
        if c == 0:
            continue
        if not wait_all:
            xa_cp[c].wait()
        start_stage(len(wblocks) + 1 + c)
        r = _dot_nt(wta[...], xa[pl.ds(s0, n), :])
        qta[:, pl.ds(s0, n)] = (r[0:D, :] * QSCALE).astype(BF)
        kv_store(r[D:D + 2 * DH, :], s0, n)

    CK = 128
    NU = NT_ * NG

    def a_w(u):
        t = u // NG
        g = u % NG
        tc = _ds(t)
        ws = []
        for j in range(4):
            if isinstance(u, int):
                rows = pl.ds(g * 128 + j * 32, 32)
            else:
                rows = pl.ds(pl.multiple_of(g * 128 + j * 32, 32), 32)
            ws.append(jnp.concatenate([qta[rows, tc], jnp.zeros((128 - DH, 128), BF)], axis=0))
        return jnp.concatenate(ws, axis=1)

    def a_fin(u, acc, l):
        u = (u + NU) % NU
        t = u // NG
        g = u % NG
        inv = 1.0 / jnp.sum(l, axis=0, keepdims=True)
        o_t = (acc * inv).astype(BF)
        blk = jnp.concatenate([o_t[:, j * 128:(j + 1) * 128] for j in range(4)], axis=0)
        oa[_ds(t), _ds(g)] = blk.T

    def a_step(b, u, m_cur, do1=True, do2=True, filler=None):
        mx = l = acc = None
        if do1:
            w = a_w(u + NB)
        for c in range(S // CK):
            rows = pl.ds(c * CK, CK)
            if filler is not None:
                filler()
            if do2:
                s_old = sa[b, rows, :]
            if do1:
                s = _dot(kpa[rows, :], w)
                sa[b, rows, :] = s
                mx = _chain(jnp.maximum, mx, s)
            if do2:
                p = jnp.exp2(s_old - m_cur)
                l = _chain(jnp.add, l, p)
                o = _dot(vta[:, rows], p.astype(BF))
                acc = o if acc is None else acc + o
        m_new = jnp.max(mx, axis=0, keepdims=True) if do1 else None
        return m_new, acc, l

    def a_multi(u0, ms, do1=True, filler=None):
        new = []
        prev = None
        for b in range(NB):
            if b == 0:
                a_fin(u0 - 1, acc_ref[...], l_ref[...])
            else:
                a_fin(u0 + b - 1, *prev)
            m, acc, l = a_step(b, u0 + b, ms[b], do1=do1, filler=filler)
            prev = (acc, l)
            new.append(m)
        acc_ref[...] = prev[0]
        l_ref[...] = prev[1]
        return new

    def make_filler(thunks, nslots):
        state = dict(i=0, k=0)

        def f():
            want = (state['i'] * len(thunks) + nslots - 1) // nslots + 1
            want = min(want, len(thunks))
            while state['k'] < want:
                thunks[state['k']]()
                state['k'] += 1
            state['i'] += 1
        f.rest = lambda: [t() for t in thunks[state['k']:]]
        return f

    scope('a_fill')
    ms = [a_step(b, b - NB, None, do2=False)[0] for b in range(NB)]
    acc_ref[...] = jnp.zeros(acc_ref.shape, F32)
    l_ref[...] = jnp.ones(l_ref.shape, F32)
    scope('a_loop')

    def a_body(i, ms):
        @pl.when(i == 1)
        def _():
            woa_cp.start()
            wqkv_cp.start()
            xb_cp.start()
            wob_cp.start()

        return tuple(a_multi(i * NB, list(ms)))

    ms = lax.fori_loop(0, NU // NB - 1, a_body, tuple(ms))

    def out_cp(src, s0, n, col0, sem):
        return cp(src.at[pl.ds(s0, n)], out_h.at[pl.ds(s0, n), pl.ds(col0, D)], sem)

    def oproj_pieces(o_ref, w_ref, dst, s0, n):
        def piece(j):
            cols = pl.ds(j * 128, 128)
            dst[pl.ds(s0, n), cols] = _dot(o_ref[pl.ds(s0, n), :], w_ref[:, cols]).astype(BF)
        return [functools.partial(piece, j) for j in range(D // 128)]

    scope('a_drain_oproj')
    woa_cp.wait()
    wqkv_cp.wait()
    xb_cp.wait()
    oa_chunks = []
    s0 = 0
    for n in OA_CH:
        oa_chunks.append((s0, n))
        s0 += n
    assert s0 == S
    outa_cps = [out_cp(outa, s0, n, 0, sem_o.at[c]) for c, (s0, n) in enumerate(oa_chunks)]
    if merge_a:
        fill = make_filler(oproj_pieces(oa, woa, outa, *oa_chunks[0]), NB * (S // CK))
        a_multi(NU - NB, list(ms), do1=False, filler=fill)
        fill.rest()
        outa_cps[0].start()
        a_fin(NU - 1, acc_ref[...], l_ref[...])
    else:
        a_multi(NU - NB, list(ms), do1=False)
        a_fin(NU - 1, acc_ref[...], l_ref[...])
        s0, n = oa_chunks[0]
        outa[pl.ds(s0, n), :] = _dot(oa[pl.ds(s0, n), :], woa[...]).astype(BF)
        outa_cps[0].start()
    for c, (s0, n) in enumerate(oa_chunks):
        if c == 0:
            continue
        outa[pl.ds(s0, n), :] = _dot(oa[pl.ds(s0, n), :], woa[...]).astype(BF)
        outa_cps[c].start()
        nper = -(-16 // (len(oa_chunks) - 1))
        for j in range((c - 1) * nper, min(16, c * nper)):
            wtb_piece(j)

    scope('b_proj')

    def proj_b(c, carry):
        cols = _ds(c, TCB)
        x = xb[cols, :]
        r = _dot_nt(wtb[pl.ds(0, D), :], x)
        qtb[:, cols] = (r * QSCALE).astype(BF)
        r = _dot_nt(wtb[pl.ds(D, D), :], x)
        vtb[:, cols] = r.astype(BF)
        kb[cols, :] = _dot(x, wqkv[:, pl.ds(D, D)]).astype(BF)
        return carry

    lax.fori_loop(0, S // TCB, proj_b, 0)

    scope('b_fill')
    row = lax.broadcasted_iota(jnp.int32, (128, 128), 0)
    col = lax.broadcasted_iota(jnp.int32, (128, 128), 1)
    bias[0] = jnp.where(row > col, 0.0, NEG).astype(F32)
    bias[1] = jnp.where(row <= col, 0.0, NEG).astype(F32)

    def b_w(t, g):
        tc = _ds(t)
        ws = []
        for j in range(4):
            parts = []
            if j > 0:
                parts.append(jnp.zeros((32 * j, 128), BF))
            parts.append(qtb[pl.ds(g * 128 + j * 32, 32), tc])
            if j < 3:
                parts.append(jnp.zeros((96 - 32 * j, 128), BF))
            ws.append(jnp.concatenate(parts, axis=0))
        return jnp.concatenate(ws, axis=1)

    def b_fin(g, t, acc, l):
        inv = 1.0 / jnp.sum(l, axis=0, keepdims=True)
        blk = jnp.concatenate([acc[j] * inv[:, j * 128:(j + 1) * 128] for j in range(4)], axis=0)
        ob[_ds(t), pl.ds(g * 128, 128)] = blk.astype(BF).T

    def b_unit(g, t2, nt2, m_cur, t1, nt1, prev, filler):
        mx = l = None
        acc = [None] * 4
        if nt1:
            w = b_w(t1, g)
        if prev is not None:
            b_fin(*prev)
        for ti in range(3):
            rows = pl.ds(ti * 128, 128)
            do2 = ti >= 3 - nt2
            do1 = ti >= 3 - nt1
            if filler is not None:
                filler()
            if do2:
                s_old = sb[g, rows, :]
            if do1:
                s = _dot(kb[_ds(t1 + ti - 2), pl.ds(g * 128, 128)], w)
                if ti != 1:
                    bt = bias[ti // 2]
                    s = s + jnp.concatenate([bt] * 4, axis=1)
                sb[g, rows, :] = s
                mx = _chain(jnp.maximum, mx, s)
            if do2:
                p = jnp.exp2(s_old - m_cur)
                l = _chain(jnp.add, l, p)
                for j in range(4):
                    o = _dot(vtb[pl.ds(g * 128 + j * 32, 32), _ds(t2 + ti - 2)],
                             p[:, j * 128:(j + 1) * 128].astype(BF))
                    acc[j] = o if acc[j] is None else acc[j] + o
        m_new = jnp.max(mx, axis=0, keepdims=True) if nt1 else None
        return m_new, ((g, t2, acc, l) if nt2 else None)

    def b_tile(t2, nt2, ms, t1, nt1, fin_prev, filler=None):
        out = []
        prev = None
        if fin_prev:
            a = acc_ref[...]
            prev = (NG - 1, t2 - 1, [a[:, j * 128:(j + 1) * 128] for j in range(4)], l_ref[...])
        for g in range(NG):
            m, prev = b_unit(g, t2, nt2, ms[g] if ms else None, t1, nt1, prev, filler)
            out.append(m)
        if prev is not None:
            acc_ref[...] = jnp.concatenate(prev[2], axis=1)
            l_ref[...] = prev[3]
        return out

    ms = b_tile(None, 0, None, 0, 1, False)
    ms = b_tile(0, 1, ms, 1, 2, False)
    ms = b_tile(1, 2, ms, 2, 3, True)
    scope('b_loop')
    ms = lax.fori_loop(2, NT_ - 1, lambda t, ms: tuple(b_tile(t, 3, list(ms), t + 1, 3, True)), tuple(ms))

    scope('b_drain_oproj')
    wob_cp.wait()
    ob_chunks = []
    s0 = 0
    for n in OB_CH:
        ob_chunks.append((s0, n))
        s0 += n
    assert s0 == S
    outb_cps = [out_cp(outb, s0, n, D, sem_o.at[len(oa_chunks) + c]) for c, (s0, n) in enumerate(ob_chunks)]

    def b_last_fin():
        a = acc_ref[...]
        b_fin(NG - 1, NT_ - 1, [a[:, j * 128:(j + 1) * 128] for j in range(4)], l_ref[...])

    if merge_b:
        fill = make_filler(oproj_pieces(ob, wob, outb, *ob_chunks[0]), NG * 3)
        b_tile(NT_ - 1, 3, list(ms), None, 0, True, filler=fill)
        fill.rest()
        outb_cps[0].start()
        b_last_fin()
    else:
        b_tile(NT_ - 1, 3, list(ms), None, 0, True)
        b_last_fin()
        s0, n = ob_chunks[0]
        outb[pl.ds(s0, n), :] = _dot(ob[pl.ds(s0, n), :], wob[...]).astype(BF)
        outb_cps[0].start()
    for c, (s0, n) in enumerate(ob_chunks):
        if c == 0:
            continue
        outb[pl.ds(s0, n), :] = _dot(ob[pl.ds(s0, n), :], wob[...]).astype(BF)
        outb_cps[c].start()
    scope('tail')
    for c in outa_cps + outb_cps:
        c.wait()
    scope(None)


def make(NB=2, MB0=(128, 384, 512), TC0=512, wait_all=True, STAGES=(('x0', 'w0', 'w1', 'w2', 'wk', 'wv', 'x1', 'x2', 'x3'),), merge_a=True, merge_b=True, OA_CH=(512, 512, 512, 512),
         OB_CH=(512, 512, 512, 384, 128), TCB=512, flags=None):
    def f(A_x, A_wq, A_wk, A_wv, A_wo, B_x, B_wqkv, B_wo):
        any_spec = pl.BlockSpec(memory_space=pl.ANY)
        V = pltpu.VMEM
        scratch = [
            V((S, D), BF), V((D, D), BF), V((D, D), BF),
            V((S, D), BF), V((D, 3 * D), BF), V((D, D), BF),
            V((D + 2 * DH, D), BF), V((2 * D, D), BF),
            V((D, S), BF), V((S, 128), BF), V((DH, S), BF), V((S, D), BF),
            V((D, S), BF), V((S, D), BF), V((D, S), BF), V((S, D), BF),
            V((NB, S, 512), F32), V((NG, 384, 512), F32), V((2, 128, 128), F32), V((DH, 512), F32), V((8, 512), F32),
            V((S, D), BF), V((S, D), BF),
            pltpu.SemaphoreType.DMA((8,)), pltpu.SemaphoreType.DMA((14,)),
            pltpu.SemaphoreType.DMA((len(OA_CH) + len(OB_CH),)),
        ]
        out = pl.pallas_call(
            functools.partial(_kernel, NB=NB, MB0=MB0, TC0=TC0, wait_all=wait_all, STAGES=STAGES, merge_a=merge_a, merge_b=merge_b,
                              OA_CH=OA_CH, OB_CH=OB_CH, TCB=TCB),
            out_shape=jax.ShapeDtypeStruct((S, 2 * D), BF),
            in_specs=[any_spec] * 8,
            out_specs=any_spec,
            scratch_shapes=scratch,
            compiler_params=pltpu.CompilerParams(vmem_limit_bytes=120 * 1024 * 1024, flags=flags),
        )(A_x.reshape(S, D), A_wq, A_wk.T, A_wv.T, A_wo, B_x.reshape(S, D), B_wqkv, B_wo)
        return out.reshape(1, S, 2 * D)
    return jax.jit(f)


_IMPL = make(STAGES=(('x0', 'w0', 'w1'), ('w2', 'wk', 'wv'), ('x1', 'x2', 'x3')))


def pallas_concat_heads__grouped_kv_mqa__sliding_block__prompt_kernel(A_x, A_wq, A_wk, A_wv, A_wo, B_x, B_wqkv, B_wo):
    return _IMPL(A_x, A_wq, A_wk, A_wv, A_wo, B_x, B_wqkv, B_wo)
```

```python
import functools
import jax
import jax.numpy as jnp
from jax import lax
import jax.experimental.pallas as pl
import jax.experimental.pallas.tpu as pltpu

S = 2048
D = 1024
H = 32
DH = 32
NG = 8
TQ = 128
NT_ = S // TQ
PROFILE = False
LOG2E = 1.4426950408889634
QSCALE = (DH ** -0.5) * LOG2E
NEG = -1e30
BF = jnp.bfloat16
F32 = jnp.float32

_NN = (((1,), (0,)), ((), ()))
_NT = (((1,), (1,)), ((), ()))


def _dot(a, b):
    return lax.dot_general(a, b, _NN, preferred_element_type=F32)


def _dot_nt(a, b):
    return lax.dot_general(a, b, _NT, preferred_element_type=F32)


def _ds(i, n=128):
    if isinstance(i, int):
        return pl.ds(i * n, n)
    return pl.ds(pl.multiple_of(i * n, n), n)


def _chain(op, acc, x):
    for r in range(x.shape[0] // 8):
        sl = x[r * 8:(r + 1) * 8, :]
        acc = sl if acc is None else op(acc, sl)
    return acc


def _tree(op, acc, x):
    xs = [x[r * 8:(r + 1) * 8, :] for r in range(x.shape[0] // 8)]
    while len(xs) > 1:
        xs = [op(xs[i], xs[i + 1]) if i + 1 < len(xs) else xs[i] for i in range(0, len(xs), 2)]
    return xs[0] if acc is None else op(acc, xs[0])


def _kernel(xa_h, wq_h, wk_h, wv_h, woa_h, xb_h, wqkv_h, wob_h, out_h,
            xa, wq, woa, xb, wqkv, wob,
            wta, wtb, qta, kpa, vta, oa, qtb, kb, vtb, ob,
            sa, sb, bias, acc_ref, l_ref, outa, outb,
            sem_x, sem_w, sem_o, *, NB, MB0, TC0, wait_all, STAGES, merge_a, merge_b, PA, PB, wtb_in_drain, TREE_DRAIN, TREE_BFILL, BUNROLL, NBB, BORD, BMT, OA_CH, OB_CH, TCB):
    def cp(src, dst, sem):
        return pltpu.make_async_copy(src, dst, sem)

    _sc = [None]
    def scope(name):
        if not PROFILE:
            return
        if _sc[0] is not None:
            _sc[0].__exit__(None, None, None)
            _sc[0] = None
        if name is not None:
            _sc[0] = jax.named_scope(name)
            _sc[0].__enter__()
    scope('issue')
    a_chunks = [(0, TC0)]
    while a_chunks[-1][0] + a_chunks[-1][1] < S:
        s0 = a_chunks[-1][0] + a_chunks[-1][1]
        a_chunks.append((s0, min(512, S - s0)))
    xa_cp = [cp(xa_h.at[pl.ds(s0, n)], xa.at[pl.ds(s0, n)], sem_x.at[c]) for c, (s0, n) in enumerate(a_chunks)]
    wblocks = []
    m0 = 0
    for n in MB0:
        wblocks.append((m0, n))
        m0 += n
    assert m0 == D
    wq_cp = [cp(wq_h.at[:, pl.ds(m0, n)], wq.at[:, pl.ds(m0, n)], sem_w.at[j]) for j, (m0, n) in enumerate(wblocks)]
    wk_cp = cp(wk_h, wta.at[pl.ds(D, DH)], sem_w.at[8])
    wv_cp = cp(wv_h, wta.at[pl.ds(D + DH, DH)], sem_w.at[9])
    wqkv_cp = cp(wqkv_h, wqkv, sem_w.at[10])
    xb_cp = cp(xb_h, xb, sem_w.at[11])
    woa_cp = cp(woa_h, woa, sem_w.at[12])
    wob_cp = cp(wob_h, wob, sem_w.at[13])

    named = {'x%d' % c: d for c, d in enumerate(xa_cp)}
    named.update({'w%d' % j: d for j, d in enumerate(wq_cp)})
    named.update(wk=wk_cp, wv=wv_cp)

    def start_stage(k):
        if k < len(STAGES):
            for nm in STAGES[k]:
                if isinstance(nm, tuple):
                    named[nm[0]].start(priority=nm[1])
                else:
                    named[nm].start()

    start_stage(0)

    def kv_store(r, s0, n):
        cols = pl.ds(s0, n)
        kt = r[0:DH, :].astype(BF)
        vta[:, cols] = r[DH:2 * DH, :].astype(BF)
        kpa[cols, :] = jnp.concatenate([kt, jnp.zeros((128 - DH, n), BF)], axis=0).T

    s0, n = a_chunks[0]
    scope('w_x0')
    xa_cp[0].wait()
    for j, (m0, mn) in enumerate(wblocks):
        scope('w_w%d' % j)
        wq_cp[j].wait()
        start_stage(j + 1)
        scope('blk%d' % j)
        x0 = xa[pl.ds(s0, n), :]
        for q in range(mn // 128):
            rows = pl.ds(m0 + q * 128, 128)
            w = wq[:, rows].T
            wta[rows, :] = w
            qta[rows, pl.ds(s0, n)] = (_dot_nt(w, x0) * QSCALE).astype(BF)
        if j == len(wblocks) - 1:
            wk_cp.wait()
            wv_cp.wait()
            kv_store(_dot_nt(wta[pl.ds(D, 2 * DH), :], x0), s0, n)
    scope('w_xrest')
    start_stage(len(wblocks) + 1)
    if wait_all:
        for c in xa_cp[1:]:
            c.wait()
    xwait = {}
    if not wait_all:
        xwait = {1: [1], 2: list(range(2, len(a_chunks)))}

    def wtb_piece(j):
        src = j * 128 if j < 8 else 2 * D + (j - 8) * 128
        wtb[pl.ds(j * 128, 128), :] = wqkv[:, pl.ds(src, 128)].T

    scope('p0_rest')
    for c, (s0, n) in enumerate(a_chunks):
        if c == 0:
            continue
        for cc in xwait.get(c, []):
            xa_cp[cc].wait()
        start_stage(len(wblocks) + 1 + c)
        r = _dot_nt(wta[...], xa[pl.ds(s0, n), :])
        qta[:, pl.ds(s0, n)] = (r[0:D, :] * QSCALE).astype(BF)
        kv_store(r[D:D + 2 * DH, :], s0, n)

    CK = 128
    NU = NT_ * NG

    def a_w(u):
        t = u // NG
        g = u % NG
        tc = _ds(t)
        ws = []
        for j in range(4):
            if isinstance(u, int):
                rows = pl.ds(g * 128 + j * 32, 32)
            else:
                rows = pl.ds(pl.multiple_of(g * 128 + j * 32, 32), 32)
            ws.append(jnp.concatenate([qta[rows, tc], jnp.zeros((128 - DH, 128), BF)], axis=0))
        return jnp.concatenate(ws, axis=1)

    def a_fin(u, acc, l):
        u = (u + NU) % NU
        t = u // NG
        g = u % NG
        inv = 1.0 / jnp.sum(l, axis=0, keepdims=True)
        o_t = (acc * inv).astype(BF)
        blk = jnp.concatenate([o_t[:, j * 128:(j + 1) * 128] for j in range(4)], axis=0)
        oa[_ds(t), _ds(g)] = blk.T

    def a_step(b, u, m_cur, do1=True, do2=True, filler=None):
        lfold = _tree if (do1 or TREE_DRAIN) else _chain
        mx = l = acc = None
        if do1:
            w = a_w(u + NB)
        for c in range(S // CK):
            rows = pl.ds(c * CK, CK)
            if filler is not None:
                filler()
            if do2:
                s_old = sa[b, rows, :]
            if do1:
                s = _dot(kpa[rows, :], w)
                sa[b, rows, :] = s
                mx = _chain(jnp.maximum, mx, s)
            if do2:
                p = jnp.exp2(s_old - m_cur)
                l = lfold(jnp.add, l, p)
                o = _dot(vta[:, rows], p.astype(BF))
                acc = o if acc is None else acc + o
        m_new = jnp.max(mx, axis=0, keepdims=True) if do1 else None
        return m_new, acc, l

    def a_multi(u0, ms, n, ndo1, filler=None):
        ms = list(ms)
        prev = None
        for i in range(n):
            b = i % NB
            if i == 0:
                a_fin(u0 - 1, acc_ref[...], l_ref[...])
            else:
                a_fin(u0 + i - 1, *prev)
            m, acc, l = a_step(b, u0 + i, ms[b], do1=i < ndo1, filler=filler)
            prev = (acc, l)
            ms[b] = m
        acc_ref[...] = prev[0]
        l_ref[...] = prev[1]
        return ms

    def make_filler(thunks, nslots):
        state = dict(i=0, k=0)

        def f():
            want = (state['i'] * len(thunks) + nslots - 1) // nslots + 1
            want = min(want, len(thunks))
            while state['k'] < want:
                thunks[state['k']]()
                state['k'] += 1
            state['i'] += 1
        f.rest = lambda: [t() for t in thunks[state['k']:]]
        return f

    scope('a_fill')
    ms = [a_step(b, b - NB, None, do2=False)[0] for b in range(NB)]
    acc_ref[...] = jnp.zeros(acc_ref.shape, F32)
    l_ref[...] = jnp.ones(l_ref.shape, F32)
    scope('a_loop')

    def a_body(i, ms):
        @pl.when(i == 1)
        def _():
            woa_cp.start()
            wqkv_cp.start()
            xb_cp.start()
            wob_cp.start()

        return tuple(a_multi(i * NB, ms, NB, NB))

    NIT = (NU - NB) // NB
    NTAIL = NU - NIT * NB
    ms = lax.fori_loop(0, NIT, a_body, tuple(ms))

    def out_cp(src, s0, n, col0, sem):
        return cp(src.at[pl.ds(s0, n)], out_h.at[pl.ds(s0, n), pl.ds(col0, D)], sem)

    def oproj_pieces(o_ref, w_ref, dst, s0, n, pm, pn):
        def piece(i, j):
            rows = pl.ds(s0 + i * pm, pm)
            cols = pl.ds(j * pn, pn)
            dst[rows, cols] = _dot(o_ref[rows, :], w_ref[:, cols]).astype(BF)
        return [functools.partial(piece, i, j) for i in range(n // pm) for j in range(D // pn)]

    scope('a_drain_oproj')
    woa_cp.wait()
    wqkv_cp.wait()
    xb_cp.wait()
    oa_chunks = []
    s0 = 0
    for n in OA_CH:
        oa_chunks.append((s0, n))
        s0 += n
    assert s0 == S
    outa_cps = [out_cp(outa, s0, n, 0, sem_o.at[c]) for c, (s0, n) in enumerate(oa_chunks)]
    if merge_a:
        nm = len(oa_chunks) - len(OA_CH) + merge_a
        pcs = []
        for c in range(merge_a):
            pcs += oproj_pieces(oa, woa, outa, *oa_chunks[c], *PA)
        if wtb_in_drain:
            step = len(pcs) // 16
            for j in range(16):
                pcs.insert(len(pcs) - j * step if False else (15 - j) * step + step // 2, functools.partial(wtb_piece, 15 - j))
        fill = make_filler(pcs, NTAIL * (S // CK))
        a_multi(NIT * NB, ms, NTAIL, NTAIL - NB, filler=fill)
        fill.rest()
        for c in range(merge_a):
            outa_cps[c].start()
        a_fin(NU - 1, acc_ref[...], l_ref[...])
    else:
        a_multi(NIT * NB, ms, NTAIL, NTAIL - NB)
        a_fin(NU - 1, acc_ref[...], l_ref[...])
        s0, n = oa_chunks[0]
        outa[pl.ds(s0, n), :] = _dot(oa[pl.ds(s0, n), :], woa[...]).astype(BF)
        outa_cps[0].start()
    first = max(1, merge_a)
    for c, (s0, n) in enumerate(oa_chunks):
        if c < first:
            continue
        outa[pl.ds(s0, n), :] = _dot(oa[pl.ds(s0, n), :], woa[...]).astype(BF)
        outa_cps[c].start()
        if not wtb_in_drain:
            nper = -(-16 // (len(oa_chunks) - first))
            for j in range((c - first) * nper, min(16, (c - first + 1) * nper)):
                wtb_piece(j)

    scope('b_proj')

    def proj_b(c, carry):
        cols = _ds(c, TCB)
        x = xb[cols, :]
        r = _dot_nt(wtb[pl.ds(0, D), :], x)
        qtb[:, cols] = (r * QSCALE).astype(BF)
        r = _dot_nt(wtb[pl.ds(D, D), :], x)
        vtb[:, cols] = r.astype(BF)
        kb[cols, :] = _dot(x, wqkv[:, pl.ds(D, D)]).astype(BF)
        return carry

    if BUNROLL:
        for c in range(S // TCB):
            proj_b(c, 0)
    else:
        lax.fori_loop(0, S // TCB, proj_b, 0)

    scope('b_fill')
    row = lax.broadcasted_iota(jnp.int32, (128, 128), 0)
    col = lax.broadcasted_iota(jnp.int32, (128, 128), 1)
    bias[0:128, :] = jnp.where(row <= col, 0.0, NEG).astype(F32)
    r = row[0:32, :]
    c = col[0:32, :] // 32
    ii = col[0:32, :] % 32
    bias[128:160, :] = jnp.where((c == 3) & (r <= ii), NEG, 0.0).astype(F32)
    bias[160:192, :] = jnp.where((c == 0) & (r > ii), NEG, 0.0).astype(F32)
    for k in range(3):
        bias[192 + 32 * k:224 + 32 * k, :] = jnp.where(
            ((c == k) & (r <= ii)) | ((c == k + 1) & (r > ii)), NEG, 0.0).astype(F32)
    B_DIAG, B_HEAD, B_TAIL, B_MRG = pl.ds(0, 128), pl.ds(128, 32), pl.ds(160, 32), pl.ds(192, 96)

    def bias4(rows):
        return jnp.concatenate([bias[rows, :]] * 4, axis=1)

    def rows_at(t, off, n):
        if isinstance(t, int):
            return pl.ds(t * 128 + off, n)
        return pl.ds(pl.multiple_of(t * 128 + off, 32), n)

    def place(parts):
        out, pos = [], 0
        for off, v in sorted(parts, key=lambda x: x[0]):
            if off > pos:
                out.append(jnp.zeros((off - pos, 128), BF))
            out.append(v)
            pos = off + 32
        if pos < 128:
            out.append(jnp.zeros((128 - pos, 128), BF))
        return jnp.concatenate(out, axis=0)

    def q_piece(t, g, j):
        return qtb[pl.ds(g * 128 + j * 32, 32), _ds(t)]

    def b_w(t, g):
        return jnp.concatenate([place([(32 * j, q_piece(t, g, j))]) for j in range(4)], axis=1)

    def b_w2(t, g, k):
        lane = lax.broadcasted_iota(jnp.int32, (16, 128), 1)
        mlo = jnp.where(lane < 32 * (k + 1), jnp.uint32(0xFFFFFFFF), jnp.uint32(0))
        ws = []
        for j in range(4):
            q = pltpu.bitcast(q_piece(t, g, j), jnp.uint32)
            qlo = pltpu.bitcast(q & mlo, BF)
            qhi = pltpu.bitcast(q & ~mlo, BF)
            if j < 2:
                ws.append(place([(32 * j, qlo), (64 + 32 * j, qhi)]))
            else:
                ws.append(place([(32 * j, qlo), (32 * (j - 2), qhi)]))
        return jnp.concatenate(ws[:2], axis=1), jnp.concatenate(ws[2:], axis=1)

    def b_fin(g, t, acc, l):
        inv = 1.0 / jnp.sum(l, axis=0, keepdims=True)
        blk = jnp.concatenate([acc[j] * inv[:, j * 128:(j + 1) * 128] for j in range(4)], axis=0)
        ob[_ds(t), pl.ds(g * 128, 128)] = blk.astype(BF).T

    lane512 = lax.broadcasted_iota(jnp.int32, (32, 512), 1) % 128
    lo_part = [lane512 < 32 * (k + 1) for k in range(3)]

    def b_unit(g, t2, nt2, m_cur, t1, nt1, prev, filler, p):
        lfold = _tree if ((nt1 and (nt2 == 3 or TREE_BFILL)) or TREE_DRAIN) else _chain
        st = dict(mx=None, l=None, acc=[None] * 4)
        gl = pl.ds(g * 128, 128)
        if prev is not None:
            b_fin(*prev)
        if nt1:
            w = b_w(t1, g)

        def put(off, s):
            sb[p * NG + g, pl.ds(off, s.shape[0]), :] = s
            st['mx'] = (_tree if BMT else _chain)(jnp.maximum, st['mx'], s)

        def qk_wide():
            s = _dot(kb[rows_at(t1, -160, 192), gl], w)
            s = jnp.concatenate([s[0:32] + bias4(B_HEAD), s[32:160], s[160:] + bias4(B_TAIL)], axis=0)
            put(96, s)

        def qk_merged():
            kf = pltpu.bitcast(kb[rows_at(t1, -256, 96), gl], jnp.uint32)
            kd = pltpu.roll(pltpu.bitcast(kb[rows_at(t1, 32, 96), gl], jnp.uint32), 64, 1)
            ln = lax.broadcasted_iota(jnp.int32, kf.shape, 1) < 64
            la = pltpu.bitcast(jnp.where(ln, kf, kd), BF)
            lb = pltpu.bitcast(jnp.where(ln, kd, kf), BF)
            parts = []
            for k in range(3):
                w2a, w2b = b_w2(t1, g, k)
                rows = slice(32 * k, 32 * k + 32)
                parts.append(jnp.concatenate([_dot(la[rows], w2a), _dot(lb[rows], w2b)], axis=1))
            put(0, jnp.concatenate(parts, axis=0) + bias4(B_MRG))

        def qk_nat(ti):
            s = _dot(kb[_ds(t1 + ti - 2), gl], w)
            if ti == 2:
                s = s + bias4(B_DIAG)
            put(ti * 128 - 96, s)

        def prob(s_old):
            p = jnp.exp2(s_old - m_cur)
            st['l'] = lfold(jnp.add, st['l'], p)
            return p

        def load(off, n):
            return sb[p * NG + g, pl.ds(off, n), :]

        def pv(ti, parts):
            for j in range(4):
                pj = jnp.concatenate([p[:, j * 128:(j + 1) * 128] for p in parts], axis=0).astype(BF)
                o = _dot(vtb[pl.ds(g * 128 + j * 32, 32), _ds(t2 + ti - 2)], pj)
                st['acc'][j] = o if st['acc'][j] is None else st['acc'][j] + o

        def fill():
            if filler is not None:
                filler()

        def pass1(k):
            if nt1 == 3:
                (qk_merged, None, qk_wide)[k] and (qk_merged, None, qk_wide)[k]()
            elif nt1 and k >= 3 - nt1:
                qk_nat(k)

        if nt2 == 3:
            inter = nt1 == 3
            fill()
            if BORD == 0 or not inter:
                sm, sf = load(0, 96), load(96, 32)
                if inter:
                    pass1(0)
                pm, pf = prob(sm), prob(sf)
                pms = [pm[32 * k:32 * k + 32] for k in range(3)]
                pv(0, [jnp.where(lo_part[k], pms[k], 0.0) for k in range(3)] + [pf])
                fill()
                smid, sd = load(128, 128), load(256, 32)
                if inter:
                    pass1(2)
                pv(1, [prob(smid)])
                fill()
                pv(2, [prob(sd)] + [jnp.where(lo_part[k], 0.0, pms[k]) for k in range(3)])
            elif BORD == 1:
                sm, sf, smid, sd = load(0, 96), load(96, 32), load(128, 128), load(256, 32)
                pass1(2)
                pm, pf = prob(sm), prob(sf)
                pms = [pm[32 * k:32 * k + 32] for k in range(3)]
                pv(0, [jnp.where(lo_part[k], pms[k], 0.0) for k in range(3)] + [pf])
                pv(1, [prob(smid)])
                pass1(0)
                pv(2, [prob(sd)] + [jnp.where(lo_part[k], 0.0, pms[k]) for k in range(3)])
            elif isinstance(BORD, str):
                sm, sf, smid, sd = load(0, 96), load(96, 32), load(128, 128), load(256, 32)
                hold = {}

                def get_pm():
                    if 'pm' not in hold:
                        pm = prob(sm)
                        hold['pm'] = [pm[32 * k:32 * k + 32] for k in range(3)]
                    return hold['pm']
                for op in BORD:
                    if op == 'w':
                        pass1(2)
                    elif op == 'm':
                        pass1(0)
                    elif op == '0':
                        pms = get_pm()
                        pv(0, [jnp.where(lo_part[k], pms[k], 0.0) for k in range(3)] + [prob(sf)])
                    elif op == '1':
                        pv(1, [prob(smid)])
                    elif op == '2':
                        pms = get_pm()
                        pv(2, [prob(sd)] + [jnp.where(lo_part[k], 0.0, pms[k]) for k in range(3)])
            elif BORD == 2:
                sm, sf, smid, sd = load(0, 96), load(96, 32), load(128, 128), load(256, 32)
                pass1(0)
                pass1(2)
                pm, pf = prob(sm), prob(sf)
                pms = [pm[32 * k:32 * k + 32] for k in range(3)]
                pv(0, [jnp.where(lo_part[k], pms[k], 0.0) for k in range(3)] + [pf])
                pv(1, [prob(smid)])
                pv(2, [prob(sd)] + [jnp.where(lo_part[k], 0.0, pms[k]) for k in range(3)])
            elif BORD == 3:
                sm, sf, smid, sd = load(0, 96), load(96, 32), load(128, 128), load(256, 32)
                pass1(0)
                pv(1, [prob(smid)])
                pass1(2)
                pm, pf = prob(sm), prob(sf)
                pms = [pm[32 * k:32 * k + 32] for k in range(3)]
                pv(0, [jnp.where(lo_part[k], pms[k], 0.0) for k in range(3)] + [pf])
                pv(2, [prob(sd)] + [jnp.where(lo_part[k], 0.0, pms[k]) for k in range(3)])
        else:
            for ti in range(3 - nt2, 3):
                pv(ti, [prob(load(ti * 128 - 96, 128))])
            for k in range(3):
                pass1(k)
        m_new = jnp.max(st['mx'], axis=0, keepdims=True) if nt1 else None
        return m_new, ((g, t2, st['acc'], st['l']) if nt2 else None)

    def ntiles(t):
        return min(t + 1, 3) if isinstance(t, int) else 3

    def b_body(t0, ms, do1=True, do2=True, fin_prev=True, filler=None):
        out = []
        prev = None
        if fin_prev:
            a = acc_ref[...]
            prev = (NG - 1, t0 - 1, [a[:, j * 128:(j + 1) * 128] for j in range(4)], l_ref[...])
        for p in range(NBB):
            t2, t1 = t0 + p, t0 + p + NBB
            for g in range(NG):
                m, prev = b_unit(g, t2, ntiles(t2) if do2 else 0, ms[p * NG + g] if do2 else None,
                                 t1, ntiles(t1) if do1 else 0, prev, filler, p)
                out.append(m)
        if prev is not None:
            acc_ref[...] = jnp.concatenate(prev[2], axis=1)
            l_ref[...] = prev[3]
        return out

    ms = b_body(-NBB, None, do2=False, fin_prev=False)
    nfirst = -(-2 // NBB)
    for i in range(nfirst):
        ms = b_body(i * NBB, ms, fin_prev=i > 0)
    scope('b_loop')
    ms = lax.fori_loop(nfirst, NT_ // NBB - 1, lambda i, ms: tuple(b_body(i * NBB, list(ms))), tuple(ms))

    scope('b_drain_oproj')
    wob_cp.wait()
    ob_chunks = []
    s0 = 0
    for n in OB_CH:
        ob_chunks.append((s0, n))
        s0 += n
    assert s0 == S
    outb_cps = [out_cp(outb, s0, n, D, sem_o.at[len(oa_chunks) + c]) for c, (s0, n) in enumerate(ob_chunks)]

    def b_last_fin():
        a = acc_ref[...]
        b_fin(NG - 1, NT_ - 1, [a[:, j * 128:(j + 1) * 128] for j in range(4)], l_ref[...])

    if merge_b:
        pcs = []
        for c in range(merge_b):
            pcs += oproj_pieces(ob, wob, outb, *ob_chunks[c], *PB)
        fill = make_filler(pcs, NG * 3 * NBB)
        b_body(NT_ - NBB, list(ms), do1=False, filler=fill)
        fill.rest()
        for c in range(merge_b):
            outb_cps[c].start()
        b_last_fin()
    else:
        b_body(NT_ - NBB, list(ms), do1=False)
        b_last_fin()
        s0, n = ob_chunks[0]
        outb[pl.ds(s0, n), :] = _dot(ob[pl.ds(s0, n), :], wob[...]).astype(BF)
        outb_cps[0].start()
    for c, (s0, n) in enumerate(ob_chunks):
        if c < max(1, merge_b):
            continue
        outb[pl.ds(s0, n), :] = _dot(ob[pl.ds(s0, n), :], wob[...]).astype(BF)
        outb_cps[c].start()
    scope('tail')
    for c in outa_cps + outb_cps:
        c.wait()
    scope(None)


def make(NB=4, MB0=(128, 128, 256, 512), TC0=512, wait_all=False, STAGES=(('x0', 'w0', 'w1'), ('w2',), ('w3', 'wk', 'wv'), ('x1',), ('x2', 'x3')), merge_a=2, merge_b=1, NBB=1, BORD=0, BMT=False, PA=(128, 128), PB=(128, 128), wtb_in_drain=False, TREE_DRAIN=False, TREE_BFILL=False, BUNROLL=False, OA_CH=(512, 512, 512, 512),
         OB_CH=(512, 512, 512, 384, 128), TCB=512, flags=None):
    def f(A_x, A_wq, A_wk, A_wv, A_wo, B_x, B_wqkv, B_wo):
        any_spec = pl.BlockSpec(memory_space=pl.ANY)
        V = pltpu.VMEM
        scratch = [
            V((S, D), BF), V((D, D), BF), V((D, D), BF),
            V((S, D), BF), V((D, 3 * D), BF), V((D, D), BF),
            V((D + 2 * DH, D), BF), V((2 * D, D), BF),
            V((D, S), BF), V((S, 128), BF), V((DH, S), BF), V((S, D), BF),
            V((D, S), BF), V((S, D), BF), V((D, S), BF), V((S, D), BF),
            V((NB, S, 512), F32), V((NBB * NG, 288, 512), F32), V((288, 128), F32), V((DH, 512), F32), V((8, 512), F32),
            V((S, D), BF), V((S, D), BF),
            pltpu.SemaphoreType.DMA((8,)), pltpu.SemaphoreType.DMA((14,)),
            pltpu.SemaphoreType.DMA((len(OA_CH) + len(OB_CH),)),
        ]
        out = pl.pallas_call(
            functools.partial(_kernel, NB=NB, MB0=MB0, TC0=TC0, wait_all=wait_all, STAGES=STAGES, merge_a=merge_a, merge_b=merge_b, PA=PA, PB=PB, wtb_in_drain=wtb_in_drain, TREE_DRAIN=TREE_DRAIN, TREE_BFILL=TREE_BFILL, BUNROLL=BUNROLL, NBB=NBB, BORD=BORD, BMT=BMT,
                              OA_CH=OA_CH, OB_CH=OB_CH, TCB=TCB),
            out_shape=jax.ShapeDtypeStruct((S, 2 * D), BF),
            in_specs=[any_spec] * 8,
            out_specs=any_spec,
            scratch_shapes=scratch,
            compiler_params=pltpu.CompilerParams(vmem_limit_bytes=120 * 1024 * 1024, flags=flags),
        )(A_x.reshape(S, D), A_wq, A_wk.T, A_wv.T, A_wo, B_x.reshape(S, D), B_wqkv, B_wo)
        return out.reshape(1, S, 2 * D)
    return jax.jit(f)


_IMPL = make(NBB=2, merge_b=2, BORD=1)


def pallas_concat_heads__grouped_kv_mqa__sliding_block__prompt_kernel(A_x, A_wq, A_wk, A_wv, A_wo, B_x, B_wqkv, B_wo):
    return _IMPL(A_x, A_wq, A_wk, A_wv, A_wo, B_x, B_wqkv, B_wo)
```

```python
import functools

import numpy as np
import jax
import jax.numpy as jnp
from jax import lax
import jax.experimental.pallas as pl
import jax.experimental.pallas.tpu as pltpu

S = 2048
D = 1024
DH = 32
NG = 8
NQ = S // 128
NU = NQ * NG
CK = 128
NB = 7
NBB = 2
XC = 512
WQ_BLOCKS = (128, 128, 256, 512)
OA_CH = (512, 512, 512, 512)
OB_CH = (512, 512, 512, 384, 128)
QSCALE = (DH ** -0.5) * 1.4426950408889634
NEG = -1e30
BF = jnp.bfloat16
F32 = jnp.float32


def _dot(a, b):
    return lax.dot_general(a, b, (((1,), (0,)), ((), ())), preferred_element_type=F32)


def _dot_nt(a, b):
    return lax.dot_general(a, b, (((1,), (1,)), ((), ())), preferred_element_type=F32)


def _ds(i, n=128):
    if isinstance(i, int):
        return pl.ds(i * n, n)
    return pl.ds(pl.multiple_of(i * n, n), n)


def _chain(op, acc, x):
    for r in range(x.shape[0] // 8):
        sl = x[r * 8:(r + 1) * 8, :]
        acc = sl if acc is None else op(acc, sl)
    return acc


def _tree(op, acc, x):
    xs = [x[r * 8:(r + 1) * 8, :] for r in range(x.shape[0] // 8)]
    while len(xs) > 1:
        xs = [op(xs[i], xs[i + 1]) if i + 1 < len(xs) else xs[i] for i in range(0, len(xs), 2)]
    return xs[0] if acc is None else op(acc, xs[0])


def _offsets(sizes):
    out, s0 = [], 0
    for n in sizes:
        out.append((s0, n))
        s0 += n
    return out


class _Filler:
    def __init__(self, thunks, nslots):
        self.thunks, self.nslots, self.calls, self.done = thunks, nslots, 0, 0

    def __call__(self):
        want = min(-(-self.calls * len(self.thunks) // self.nslots) + 1, len(self.thunks))
        while self.done < want:
            self.thunks[self.done]()
            self.done += 1
        self.calls += 1

    def finish(self):
        while self.done < len(self.thunks):
            self.thunks[self.done]()
            self.done += 1


def _kernel(xa_h, wq_h, wkt_h, wvt_h, woa_h, xb_h, wqkv_h, wob_h, out_h,
            xa, wq, woa, xb, wqkv, wob, wta, wtb, qta, kpa, vta, oa, kb, vtb,
            sa, sb, bias, acc_ref, l_ref, sem_x, sem_w, sem_o):
    qtb, ob, outa, outb = qta, oa, xa, xb

    cp = pltpu.make_async_copy
    xa_cp = [cp(xa_h.at[pl.ds(c * XC, XC)], xa.at[pl.ds(c * XC, XC)], sem_x.at[c]) for c in range(S // XC)]
    wblocks = _offsets(WQ_BLOCKS)
    wq_cp = [cp(wq_h.at[:, pl.ds(m0, n)], wq.at[:, pl.ds(m0, n)], sem_w.at[j]) for j, (m0, n) in enumerate(wblocks)]
    wk_cp = cp(wkt_h, wta.at[pl.ds(D, DH)], sem_w.at[4])
    wv_cp = cp(wvt_h, wta.at[pl.ds(D + DH, DH)], sem_w.at[5])
    wqkv_cp = cp(wqkv_h, wqkv, sem_w.at[6])
    xb_cp = cp(xb_h, xb, sem_w.at[7])
    woa_cp = cp(woa_h, woa, sem_w.at[8])
    wob_cp = cp(wob_h, wob, sem_w.at[9])
    stages = [[xa_cp[0], wq_cp[0], wq_cp[1]], [wq_cp[2]], [wq_cp[3], wk_cp, wv_cp], [xa_cp[1]], xa_cp[2:]]

    def start(k):
        for c in stages[k]:
            c.start()

    def kv_store(r, s0, n):
        cols = pl.ds(s0, n)
        kt = r[0:DH, :].astype(BF)
        vta[:, cols] = r[DH:2 * DH, :].astype(BF)
        kpa[cols, :] = jnp.concatenate([kt, jnp.zeros((128 - DH, n), BF)], axis=0).T

    start(0)
    xa_cp[0].wait()
    for j, (m0, mn) in enumerate(wblocks):
        wq_cp[j].wait()
        start(j + 1)
        x0 = xa[pl.ds(0, XC), :]
        for q in range(mn // 128):
            rows = pl.ds(m0 + q * 128, 128)
            w = wq[:, rows].T
            wta[rows, :] = w
            qta[rows, pl.ds(0, XC)] = (_dot_nt(w, x0) * QSCALE).astype(BF)
        if j == len(wblocks) - 1:
            wk_cp.wait()
            wv_cp.wait()
            kv_store(_dot_nt(wta[pl.ds(D, 2 * DH), :], x0), 0, XC)
    for c in range(1, S // XC):
        for w_ in (xa_cp[1:2] if c == 1 else xa_cp[2:] if c == 2 else []):
            w_.wait()
        r = _dot_nt(wta[...], xa[pl.ds(c * XC, XC), :])
        qta[:, pl.ds(c * XC, XC)] = (r[0:D, :] * QSCALE).astype(BF)
        kv_store(r[D:D + 2 * DH, :], c * XC, XC)

    def a_w(u):
        t, g = u // NG, u % NG
        tc = _ds(t)
        ws = []
        for j in range(4):
            if isinstance(u, int):
                rows = pl.ds(g * 128 + j * 32, 32)
            else:
                rows = pl.ds(pl.multiple_of(g * 128 + j * 32, 32), 32)
            ws.append(jnp.concatenate([qta[rows, tc], jnp.zeros((128 - DH, 128), BF)], axis=0))
        return jnp.concatenate(ws, axis=1)

    def a_fin(u, acc, l):
        u = (u + NU) % NU
        t, g = u // NG, u % NG
        inv = 1.0 / jnp.sum(l, axis=0, keepdims=True)
        o_t = (acc * inv).astype(BF)
        blk = jnp.concatenate([o_t[:, j * 128:(j + 1) * 128] for j in range(4)], axis=0)
        oa[_ds(t), _ds(g)] = blk.T

    def a_step(b, u, m_cur, do1=True, do2=True, filler=None):
        lfold = _tree if do1 else _chain
        mx = l = acc = None
        if do1:
            w = a_w(u + NB)
        for c in range(S // CK):
            rows = pl.ds(c * CK, CK)
            if filler is not None:
                filler()
            if do2:
                s_old = sa[b, rows, :]
            if do1:
                s = _dot(kpa[rows, :], w)
                sa[b, rows, :] = s
                mx = _chain(jnp.maximum, mx, s)
            if do2:
                p = jnp.exp2(s_old - m_cur)
                l = lfold(jnp.add, l, p)
                o = _dot(vta[:, rows], p.astype(BF))
                acc = o if acc is None else acc + o
        m_new = jnp.max(mx, axis=0, keepdims=True) if do1 else None
        return m_new, acc, l

    def a_multi(u0, ms, n, ndo1, filler=None):
        ms = list(ms)
        prev = None
        for i in range(n):
            b = i % NB
            if i == 0:
                a_fin(u0 - 1, acc_ref[...], l_ref[...])
            else:
                a_fin(u0 + i - 1, *prev)
            m, acc, l = a_step(b, u0 + i, ms[b], do1=i < ndo1, filler=filler)
            prev = (acc, l)
            ms[b] = m
        acc_ref[...] = prev[0]
        l_ref[...] = prev[1]
        return ms

    ms = [a_step(b, b - NB, None, do2=False)[0] for b in range(NB)]
    acc_ref[...] = jnp.zeros(acc_ref.shape, F32)
    l_ref[...] = jnp.ones(l_ref.shape, F32)

    def a_body(i, ms):
        @pl.when(i == 1)
        def _():
            woa_cp.start()
            wqkv_cp.start()
            xb_cp.start()
            wob_cp.start()

        return tuple(a_multi(i * NB, ms, NB, NB))

    n_it = (NU - NB) // NB
    n_tail = NU - n_it * NB
    ms = lax.fori_loop(0, n_it, a_body, tuple(ms))

    def out_copies(src, chunks, col0, sem0):
        return [cp(src.at[pl.ds(s0, n)], out_h.at[pl.ds(s0, n), pl.ds(col0, D)], sem_o.at[sem0 + c])
                for c, (s0, n) in enumerate(chunks)]

    def oproj_pieces(o_ref, w_ref, dst, s0, n):
        part = {}

        def piece(i, j, h):
            rows, cols, ks = pl.ds(s0 + i * 128, 128), pl.ds(j * 256, 256), pl.ds(h * 128, 128)
            r = _dot(o_ref[rows, ks], w_ref[ks, cols])
            if h > 0:
                r = part.pop((i, j)) + r
            if h == D // 128 - 1:
                dst[rows, cols] = r.astype(BF)
            else:
                part[(i, j)] = r
        return [functools.partial(piece, i, j, h)
                for i in range(n // 128) for j in range(D // 256) for h in range(D // 128)]

    def wtb_piece(j):
        src = j * 128 if j < 8 else 2 * D + (j - 8) * 128
        wtb[pl.ds(j * 128, 128), :] = wqkv[:, pl.ds(src, 128)].T

    woa_cp.wait()
    wqkv_cp.wait()
    xb_cp.wait()
    oa_chunks = _offsets(OA_CH)
    outa_cps = out_copies(outa, oa_chunks, 0, 0)
    fill = _Filler([p for s0, n in oa_chunks[:3] for p in oproj_pieces(oa, woa, outa, s0, n)], n_tail * (S // CK))
    a_multi(n_it * NB, ms, n_tail, n_tail - NB, filler=fill)
    fill.finish()
    for c in outa_cps[:3]:
        c.start()
    a_fin(NU - 1, acc_ref[...], l_ref[...])
    s0, n = oa_chunks[3]
    outa[pl.ds(s0, n), :] = _dot(oa[pl.ds(s0, n), :], woa[...]).astype(BF)
    outa_cps[3].start()
    for j in range(16):
        wtb_piece(j)

    def proj_b(c, carry):
        cols = _ds(c, XC)
        x = xb[cols, :]
        r = _dot_nt(wtb[pl.ds(0, D), :], x)
        qtb[:, cols] = (r * QSCALE).astype(BF)
        r = _dot_nt(wtb[pl.ds(D, D), :], x)
        vtb[:, cols] = r.astype(BF)
        kb[cols, :] = _dot(x, wqkv[:, pl.ds(D, D)]).astype(BF)
        return carry

    lax.fori_loop(0, S // XC, proj_b, 0)

    row = lax.broadcasted_iota(jnp.int32, (128, 128), 0)
    col = lax.broadcasted_iota(jnp.int32, (128, 128), 1)
    bias[0:128, :] = jnp.where(row <= col, 0.0, NEG).astype(F32)
    jj = row[0:32, :]
    qb = col[0:32, :] // 32
    ii = col[0:32, :] % 32
    bias[128:160, :] = jnp.where((qb == 3) & (jj <= ii), NEG, 0.0).astype(F32)
    bias[160:192, :] = jnp.where((qb == 0) & (jj > ii), NEG, 0.0).astype(F32)
    for k in range(3):
        bias[192 + 32 * k:224 + 32 * k, :] = jnp.where(
            ((qb == k) & (jj <= ii)) | ((qb == k + 1) & (jj > ii)), NEG, 0.0).astype(F32)
    B_DIAG, B_HEAD, B_TAIL, B_MRG = pl.ds(0, 128), pl.ds(128, 32), pl.ds(160, 32), pl.ds(192, 96)

    def bias4(rows):
        return jnp.concatenate([bias[rows, :]] * 4, axis=1)

    def rows_at(t, off, n):
        if isinstance(t, int):
            return pl.ds(t * 128 + off, n)
        return pl.ds(pl.multiple_of(t * 128 + off, 32), n)

    def place(parts):
        out, pos = [], 0
        for off, v in sorted(parts, key=lambda x: x[0]):
            if off > pos:
                out.append(jnp.zeros((off - pos, 128), BF))
            out.append(v)
            pos = off + 32
        if pos < 128:
            out.append(jnp.zeros((128 - pos, 128), BF))
        return jnp.concatenate(out, axis=0)

    def q_piece(t, g, j):
        return qtb[pl.ds(g * 128 + j * 32, 32), _ds(t)]

    def b_w(t, g):
        return jnp.concatenate([place([(32 * j, q_piece(t, g, j))]) for j in range(4)], axis=1)

    def b_w2(t, g, k):
        lane = lax.broadcasted_iota(jnp.int32, (16, 128), 1)
        mlo = jnp.where(lane < 32 * (k + 1), np.uint32(0xFFFFFFFF), np.uint32(0))
        ws = []
        for j in range(4):
            q = pltpu.bitcast(q_piece(t, g, j), jnp.uint32)
            qlo = pltpu.bitcast(q & mlo, BF)
            qhi = pltpu.bitcast(q & ~mlo, BF)
            if j < 2:
                ws.append(place([(32 * j, qlo), (64 + 32 * j, qhi)]))
            else:
                ws.append(place([(32 * j, qlo), (32 * (j - 2), qhi)]))
        return jnp.concatenate(ws[:2], axis=1), jnp.concatenate(ws[2:], axis=1)

    def b_fin(g, t, acc, l):
        inv = 1.0 / jnp.sum(l, axis=0, keepdims=True)
        blk = jnp.concatenate([acc[j] * inv[:, j * 128:(j + 1) * 128] for j in range(4)], axis=0)
        ob[_ds(t), pl.ds(g * 128, 128)] = blk.astype(BF).T

    lane512 = lax.broadcasted_iota(jnp.int32, (32, 512), 1) % 128
    early = [lane512 < 32 * (k + 1) for k in range(3)]

    def b_unit(p, g, t2, nt2, m_cur, t1, nt1, prev, filler):
        lfold = _tree if (nt1 and nt2 == 3) else _chain
        st = dict(mx=None, l=None, acc=[None] * 4)
        gl = pl.ds(g * 128, 128)
        if prev is not None:
            b_fin(*prev)
        if nt1:
            w = b_w(t1, g)

        def put(off, s):
            sb[p * NG + g, pl.ds(off, s.shape[0]), :] = s
            st['mx'] = _chain(jnp.maximum, st['mx'], s)

        def load(off, n):
            return sb[p * NG + g, pl.ds(off, n), :]

        def qk_wide():
            s = _dot(kb[rows_at(t1, -160, 192), gl], w)
            put(96, jnp.concatenate([s[0:32] + bias4(B_HEAD), s[32:160], s[160:] + bias4(B_TAIL)], axis=0))

        def qk_merged():
            kf = pltpu.bitcast(kb[rows_at(t1, -256, 96), gl], jnp.uint32)
            kd = pltpu.roll(pltpu.bitcast(kb[rows_at(t1, 32, 96), gl], jnp.uint32), 64, 1)
            ln = lax.broadcasted_iota(jnp.int32, kf.shape, 1) < 64
            la = pltpu.bitcast(jnp.where(ln, kf, kd), BF)
            lb = pltpu.bitcast(jnp.where(ln, kd, kf), BF)
            parts = []
            for k in range(3):
                w2a, w2b = b_w2(t1, g, k)
                rows = slice(32 * k, 32 * k + 32)
                parts.append(jnp.concatenate([_dot(la[rows], w2a), _dot(lb[rows], w2b)], axis=1))
            put(0, jnp.concatenate(parts, axis=0) + bias4(B_MRG))

        def qk_plain(ti):
            s = _dot(kb[_ds(t1 + ti - 2), gl], w)
            if ti == 2:
                s = s + bias4(B_DIAG)
            put(ti * 128 - 96, s)

        def prob(s_old):
            pr = jnp.exp2(s_old - m_cur)
            st['l'] = lfold(jnp.add, st['l'], pr)
            return pr

        def pv(ti, parts):
            for j in range(4):
                pj = jnp.concatenate([x[:, j * 128:(j + 1) * 128] for x in parts], axis=0).astype(BF)
                o = _dot(vtb[pl.ds(g * 128 + j * 32, 32), _ds(t2 + ti - 2)], pj)
                st['acc'][j] = o if st['acc'][j] is None else st['acc'][j] + o

        def fill():
            if filler is not None:
                filler()

        def far_parts(pms, pf):
            return [jnp.where(early[k], pms[k], 0.0) for k in range(3)] + [pf]

        def diag_parts(pms, pd):
            return [pd] + [jnp.where(early[k], 0.0, pms[k]) for k in range(3)]

        def split(pm):
            return [pm[32 * k:32 * k + 32] for k in range(3)]

        if nt2 == 3 and nt1 == 3:
            sm, sf, smid, sd = load(0, 96), load(96, 32), load(128, 128), load(256, 32)
            qk_wide()
            pm, pf = prob(sm), prob(sf)
            pms = split(pm)
            pv(0, far_parts(pms, pf))
            pv(1, [prob(smid)])
            qk_merged()
            pv(2, diag_parts(pms, prob(sd)))
        elif nt2 == 3:
            fill()
            sm, sf = load(0, 96), load(96, 32)
            pm, pf = prob(sm), prob(sf)
            pms = split(pm)
            pv(0, far_parts(pms, pf))
            fill()
            smid, sd = load(128, 128), load(256, 32)
            pv(1, [prob(smid)])
            fill()
            pv(2, diag_parts(pms, prob(sd)))
        else:
            for ti in range(3 - nt2, 3):
                pv(ti, [prob(load(ti * 128 - 96, 128))])
            if nt1 == 3:
                qk_merged()
                qk_wide()
            else:
                for ti in range(3 - nt1, 3):
                    qk_plain(ti)
        m_new = jnp.max(st['mx'], axis=0, keepdims=True) if nt1 else None
        return m_new, ((g, t2, st['acc'], st['l']) if nt2 else None)

    def ntiles(t):
        return min(t + 1, 3) if isinstance(t, int) else 3

    def acc_parts():
        a = acc_ref[...]
        return [a[:, j * 128:(j + 1) * 128] for j in range(4)]

    def b_body(t0, ms, do1=True, do2=True, fin_prev=True, filler=None):
        out = []
        prev = None
        if fin_prev:
            prev = (NG - 1, t0 - 1, acc_parts(), l_ref[...])
        for p in range(NBB):
            t2, t1 = t0 + p, t0 + p + NBB
            for g in range(NG):
                m, prev = b_unit(p, g, t2, ntiles(t2) if do2 else 0, ms[p * NG + g] if do2 else None,
                                 t1, ntiles(t1) if do1 else 0, prev, filler)
                out.append(m)
        if prev is not None:
            acc_ref[...] = jnp.concatenate(prev[2], axis=1)
            l_ref[...] = prev[3]
        return out

    ms = b_body(-NBB, None, do2=False, fin_prev=False)
    ms = b_body(0, ms, fin_prev=False)
    ms = lax.fori_loop(1, NQ // NBB - 1, lambda i, ms: tuple(b_body(i * NBB, list(ms))), tuple(ms))

    wob_cp.wait()
    ob_chunks = _offsets(OB_CH)
    outb_cps = out_copies(outb, ob_chunks, D, len(oa_chunks))
    fill = _Filler(oproj_pieces(ob, wob, outb, *ob_chunks[0]), NG * 3 * NBB)
    b_body(NQ - NBB, list(ms), do1=False, filler=fill)
    fill.finish()
    outb_cps[0].start()
    b_fin(NG - 1, NQ - 1, acc_parts(), l_ref[...])
    for c, (s0, n) in enumerate(ob_chunks):
        if c == 0:
            continue
        outb[pl.ds(s0, n), :] = _dot(ob[pl.ds(s0, n), :], wob[...]).astype(BF)
        outb_cps[c].start()
    for c in outa_cps + outb_cps:
        c.wait()


@jax.jit
def pallas_concat_heads__grouped_kv_mqa__sliding_block__prompt_kernel(
    A_x: jax.Array,
    A_wq: jax.Array,
    A_wk: jax.Array,
    A_wv: jax.Array,
    A_wo: jax.Array,
    B_x: jax.Array,
    B_wqkv: jax.Array,
    B_wo: jax.Array,
):
    any_spec = pl.BlockSpec(memory_space=pl.ANY)
    V = pltpu.VMEM
    scratch = [
        V((S, D), BF), V((D, D), BF), V((D, D), BF),
        V((S, D), BF), V((D, 3 * D), BF), V((D, D), BF),
        V((D + 2 * DH, D), BF), V((2 * D, D), BF),
        V((D, S), BF), V((S, 128), BF), V((DH, S), BF), V((S, D), BF),
        V((S, D), BF), V((D, S), BF),
        V((NB, S, 512), F32), V((NBB * NG, 288, 512), F32), V((288, 128), F32),
        V((DH, 512), F32), V((8, 512), F32),
        pltpu.SemaphoreType.DMA((S // XC,)), pltpu.SemaphoreType.DMA((10,)),
        pltpu.SemaphoreType.DMA((len(OA_CH) + len(OB_CH),)),
    ]
    out = pl.pallas_call(
        _kernel,
        out_shape=jax.ShapeDtypeStruct((S, 2 * D), BF),
        in_specs=[any_spec] * 8,
        out_specs=any_spec,
        scratch_shapes=scratch,
        compiler_params=pltpu.CompilerParams(vmem_limit_bytes=112 * 1024 * 1024),
    )(A_x.reshape(S, D), A_wq, A_wk.T, A_wv.T, A_wo, B_x.reshape(S, D), B_wqkv, B_wo)
    return out.reshape(1, S, 2 * D)
```

```python
import functools

import numpy as np
import jax
import jax.numpy as jnp
from jax import lax
import jax.experimental.pallas as pl
import jax.experimental.pallas.tpu as pltpu

S = 2048
D = 1024
DH = 32
NG = 8
NQ = S // 128
NU = NQ * NG
CK = 128
NB = 7
NBB = 2
XC = 512
WQ_BLOCKS = (128, 128, 256, 512)
OA_CH = (512, 512, 512, 512)
OB_CH = (512, 512, 512, 384, 128)
QSCALE = (DH ** -0.5) * 1.4426950408889634
NEG = -1e30
BF = jnp.bfloat16
F32 = jnp.float32


def _dot(a, b):
    return lax.dot_general(a, b, (((1,), (0,)), ((), ())), preferred_element_type=F32)


def _dot_nt(a, b):
    return lax.dot_general(a, b, (((1,), (1,)), ((), ())), preferred_element_type=F32)


def _ds(i, n=128):
    if isinstance(i, int):
        return pl.ds(i * n, n)
    return pl.ds(pl.multiple_of(i * n, n), n)


def _chain(op, acc, x):
    for r in range(x.shape[0] // 8):
        sl = x[r * 8:(r + 1) * 8, :]
        acc = sl if acc is None else op(acc, sl)
    return acc


def _tree(op, acc, x):
    xs = [x[r * 8:(r + 1) * 8, :] for r in range(x.shape[0] // 8)]
    while len(xs) > 1:
        xs = [op(xs[i], xs[i + 1]) if i + 1 < len(xs) else xs[i] for i in range(0, len(xs), 2)]
    return xs[0] if acc is None else op(acc, xs[0])


def _offsets(sizes):
    out, s0 = [], 0
    for n in sizes:
        out.append((s0, n))
        s0 += n
    return out


class _Filler:
    def __init__(self, thunks, nslots):
        self.thunks, self.nslots, self.calls, self.done = thunks, nslots, 0, 0

    def __call__(self):
        want = min(-(-self.calls * len(self.thunks) // self.nslots) + 1, len(self.thunks))
        while self.done < want:
            self.thunks[self.done]()
            self.done += 1
        self.calls += 1

    def finish(self):
        while self.done < len(self.thunks):
            self.thunks[self.done]()
            self.done += 1


def _kernel(xa_h, wq_h, wkt_h, wvt_h, woa_h, xb_h, wqkv_h, wob_h, out_h,
            xa, wq, woa, xb, wqkv, wob, wta, wtb, qta, kpa, vta, oa, kb, vtb,
            sa, sb, bias, acc_ref, l_ref, sem_x, sem_w, sem_o):
    qtb, ob, outa, outb = qta, oa, xa, xb

    cp = pltpu.make_async_copy
    xa_cp = [cp(xa_h.at[pl.ds(c * XC, XC)], xa.at[pl.ds(c * XC, XC)], sem_x.at[c]) for c in range(S // XC)]
    wblocks = _offsets(WQ_BLOCKS)
    wq_cp = [cp(wq_h.at[:, pl.ds(m0, n)], wq.at[:, pl.ds(m0, n)], sem_w.at[j]) for j, (m0, n) in enumerate(wblocks)]
    wk_cp = cp(wkt_h, wta.at[pl.ds(D, DH)], sem_w.at[4])
    wv_cp = cp(wvt_h, wta.at[pl.ds(D + DH, DH)], sem_w.at[5])
    wqkv_cp = cp(wqkv_h, wqkv, sem_w.at[6])
    xb_cp = cp(xb_h, xb, sem_w.at[7])
    woa_cp = cp(woa_h, woa, sem_w.at[8])
    wob_cp = cp(wob_h, wob, sem_w.at[9])
    stages = [[xa_cp[0], wq_cp[0], wq_cp[1]], [wq_cp[2]], [wq_cp[3], wk_cp, wv_cp], [xa_cp[1]], xa_cp[2:]]

    def start(k):
        for c in stages[k]:
            c.start()

    def kv_store(r, s0, n):
        cols = pl.ds(s0, n)
        kt = r[0:DH, :].astype(BF)
        vta[:, cols] = r[DH:2 * DH, :].astype(BF)
        kpa[cols, :] = jnp.concatenate([kt, jnp.zeros((128 - DH, n), BF)], axis=0).T

    pending = []

    def flush():
        while pending:
            pending.pop(0)()

    def q_store(r, rows, cols):
        qta[rows, cols] = (r * QSCALE).astype(BF)

    start(0)
    xa_cp[0].wait()
    for j, (m0, mn) in enumerate(wblocks):
        wq_cp[j].wait()
        start(j + 1)
        flush()
        x0 = xa[pl.ds(0, XC), :]
        for q in range(mn // 128):
            rows = pl.ds(m0 + q * 128, 128)
            w = wq[:, rows].T
            wta[rows, :] = w
            flush()
            pending.append(functools.partial(q_store, _dot_nt(w, x0), rows, pl.ds(0, XC)))
        if j == len(wblocks) - 1:
            wk_cp.wait()
            wv_cp.wait()
            flush()
            pending.append(functools.partial(kv_store, _dot_nt(wta[pl.ds(D, 2 * DH), :], x0), 0, XC))
    for c in range(1, S // XC):
        for w_ in (xa_cp[1:2] if c == 1 else xa_cp[2:] if c == 2 else []):
            w_.wait()
        flush()
        r = _dot_nt(wta[...], xa[pl.ds(c * XC, XC), :])
        pending.append(functools.partial(q_store, r[0:D, :], pl.ds(0, D), pl.ds(c * XC, XC)))
        pending.append(functools.partial(kv_store, r[D:D + 2 * DH, :], c * XC, XC))
    flush()

    def a_w(u):
        t, g = u // NG, u % NG
        tc = _ds(t)
        ws = []
        for j in range(4):
            if isinstance(u, int):
                rows = pl.ds(g * 128 + j * 32, 32)
            else:
                rows = pl.ds(pl.multiple_of(g * 128 + j * 32, 32), 32)
            ws.append(jnp.concatenate([qta[rows, tc], jnp.zeros((128 - DH, 128), BF)], axis=0))
        return jnp.concatenate(ws, axis=1)

    def a_fin(u, acc, l):
        u = (u + NU) % NU
        t, g = u // NG, u % NG
        inv = 1.0 / jnp.sum(l, axis=0, keepdims=True)
        o_t = (acc * inv).astype(BF)
        blk = jnp.concatenate([o_t[:, j * 128:(j + 1) * 128] for j in range(4)], axis=0)
        oa[_ds(t), _ds(g)] = blk.T

    def a_step(b, u, m_cur, do1=True, do2=True, filler=None):
        lfold = _tree if do1 else _chain
        mx = l = acc = None
        if do1:
            w = a_w(u + NB)
        for c in range(S // CK):
            rows = pl.ds(c * CK, CK)
            if filler is not None:
                filler()
            if do2:
                s_old = sa[b, rows, :]
            if do1:
                s = _dot(kpa[rows, :], w)
                sa[b, rows, :] = s
                mx = _chain(jnp.maximum, mx, s)
            if do2:
                p = jnp.exp2(s_old - m_cur)
                l = lfold(jnp.add, l, p)
                o = _dot(vta[:, rows], p.astype(BF))
                acc = o if acc is None else acc + o
        m_new = jnp.max(mx, axis=0, keepdims=True) if do1 else None
        return m_new, acc, l

    def a_multi(u0, ms, n, ndo1, filler=None):
        ms = list(ms)
        prev = None
        for i in range(n):
            b = i % NB
            if i == 0:
                a_fin(u0 - 1, acc_ref[...], l_ref[...])
            else:
                a_fin(u0 + i - 1, *prev)
            m, acc, l = a_step(b, u0 + i, ms[b], do1=i < ndo1, filler=filler)
            prev = (acc, l)
            ms[b] = m
        acc_ref[...] = prev[0]
        l_ref[...] = prev[1]
        return ms

    ms = [a_step(b, b - NB, None, do2=False)[0] for b in range(NB)]
    acc_ref[...] = jnp.zeros(acc_ref.shape, F32)
    l_ref[...] = jnp.ones(l_ref.shape, F32)

    def a_body(i, ms):
        @pl.when(i == 1)
        def _():
            woa_cp.start()
            wqkv_cp.start()
            xb_cp.start()
            wob_cp.start()

        return tuple(a_multi(i * NB, ms, NB, NB))

    n_it = (NU - NB) // NB
    n_tail = NU - n_it * NB
    ms = lax.fori_loop(0, n_it, a_body, tuple(ms))

    def out_copies(src, chunks, col0, sem0):
        return [cp(src.at[pl.ds(s0, n)], out_h.at[pl.ds(s0, n), pl.ds(col0, D)], sem_o.at[sem0 + c])
                for c, (s0, n) in enumerate(chunks)]

    def oproj_pieces(o_ref, w_ref, dst, s0, n):
        part = {}

        def piece(i, j, h):
            rows, cols, ks = pl.ds(s0 + i * 128, 128), pl.ds(j * 256, 256), pl.ds(h * 128, 128)
            r = _dot(o_ref[rows, ks], w_ref[ks, cols])
            if h > 0:
                r = part.pop((i, j)) + r
            if h == D // 128 - 1:
                dst[rows, cols] = r.astype(BF)
            else:
                part[(i, j)] = r
        return [functools.partial(piece, i, j, h)
                for i in range(n // 128) for j in range(D // 256) for h in range(D // 128)]

    def wtb_piece(j):
        src = j * 128 if j < 8 else 2 * D + (j - 8) * 128
        wtb[pl.ds(j * 128, 128), :] = wqkv[:, pl.ds(src, 128)].T

    woa_cp.wait()
    wqkv_cp.wait()
    xb_cp.wait()
    oa_chunks = _offsets(OA_CH)
    outa_cps = out_copies(outa, oa_chunks, 0, 0)
    fill = _Filler([p for s0, n in oa_chunks[:3] for p in oproj_pieces(oa, woa, outa, s0, n)], n_tail * (S // CK))
    a_multi(n_it * NB, ms, n_tail, n_tail - NB, filler=fill)
    fill.finish()
    for c in outa_cps[:3]:
        c.start()
    a_fin(NU - 1, acc_ref[...], l_ref[...])
    s0, n = oa_chunks[3]
    outa[pl.ds(s0, n), :] = _dot(oa[pl.ds(s0, n), :], woa[...]).astype(BF)
    outa_cps[3].start()
    for j in range(16):
        wtb_piece(j)

    def proj_b(c, carry):
        cols = _ds(c, XC)
        x = xb[cols, :]
        r = _dot_nt(wtb[pl.ds(0, D), :], x)
        qtb[:, cols] = (r * QSCALE).astype(BF)
        r = _dot_nt(wtb[pl.ds(D, D), :], x)
        vtb[:, cols] = r.astype(BF)
        kb[cols, :] = _dot(x, wqkv[:, pl.ds(D, D)]).astype(BF)
        return carry

    lax.fori_loop(0, S // XC, proj_b, 0)

    row = lax.broadcasted_iota(jnp.int32, (128, 128), 0)
    col = lax.broadcasted_iota(jnp.int32, (128, 128), 1)
    bias[0:128, :] = jnp.where(row <= col, 0.0, NEG).astype(F32)
    jj = row[0:32, :]
    qb = col[0:32, :] // 32
    ii = col[0:32, :] % 32
    bias[128:160, :] = jnp.where((qb == 3) & (jj <= ii), NEG, 0.0).astype(F32)
    bias[160:192, :] = jnp.where((qb == 0) & (jj > ii), NEG, 0.0).astype(F32)
    for k in range(3):
        bias[192 + 32 * k:224 + 32 * k, :] = jnp.where(
            ((qb == k) & (jj <= ii)) | ((qb == k + 1) & (jj > ii)), NEG, 0.0).astype(F32)
    B_DIAG, B_HEAD, B_TAIL, B_MRG = pl.ds(0, 128), pl.ds(128, 32), pl.ds(160, 32), pl.ds(192, 96)

    def bias4(rows):
        return jnp.concatenate([bias[rows, :]] * 4, axis=1)

    def rows_at(t, off, n):
        if isinstance(t, int):
            return pl.ds(t * 128 + off, n)
        return pl.ds(pl.multiple_of(t * 128 + off, 32), n)

    def place(parts):
        out, pos = [], 0
        for off, v in sorted(parts, key=lambda x: x[0]):
            if off > pos:
                out.append(jnp.zeros((off - pos, 128), BF))
            out.append(v)
            pos = off + 32
        if pos < 128:
            out.append(jnp.zeros((128 - pos, 128), BF))
        return jnp.concatenate(out, axis=0)

    def q_piece(t, g, j):
        return qtb[pl.ds(g * 128 + j * 32, 32), _ds(t)]

    def b_w(t, g):
        return jnp.concatenate([place([(32 * j, q_piece(t, g, j))]) for j in range(4)], axis=1)

    def b_w2(t, g, k):
        lane = lax.broadcasted_iota(jnp.int32, (16, 128), 1)
        mlo = jnp.where(lane < 32 * (k + 1), np.uint32(0xFFFFFFFF), np.uint32(0))
        ws = []
        for j in range(4):
            q = pltpu.bitcast(q_piece(t, g, j), jnp.uint32)
            qlo = pltpu.bitcast(q & mlo, BF)
            qhi = pltpu.bitcast(q & ~mlo, BF)
            if j < 2:
                ws.append(place([(32 * j, qlo), (64 + 32 * j, qhi)]))
            else:
                ws.append(place([(32 * j, qlo), (32 * (j - 2), qhi)]))
        return jnp.concatenate(ws[:2], axis=1), jnp.concatenate(ws[2:], axis=1)

    def b_fin(g, t, acc, l):
        inv = 1.0 / jnp.sum(l, axis=0, keepdims=True)
        blk = jnp.concatenate([acc[j] * inv[:, j * 128:(j + 1) * 128] for j in range(4)], axis=0)
        ob[_ds(t), pl.ds(g * 128, 128)] = blk.astype(BF).T

    lane512 = lax.broadcasted_iota(jnp.int32, (32, 512), 1) % 128
    early = [lane512 < 32 * (k + 1) for k in range(3)]

    def b_unit(p, g, t2, nt2, m_cur, t1, nt1, prev, filler):
        lfold = _tree if (nt1 and nt2 == 3) else _chain
        st = dict(mx=None, l=None, acc=[None] * 4)
        gl = pl.ds(g * 128, 128)
        if prev is not None:
            b_fin(*prev)
        if nt1:
            w = b_w(t1, g)

        def put(off, s):
            sb[p * NG + g, pl.ds(off, s.shape[0]), :] = s
            st['mx'] = _chain(jnp.maximum, st['mx'], s)

        def load(off, n):
            return sb[p * NG + g, pl.ds(off, n), :]

        def qk_wide():
            s = _dot(kb[rows_at(t1, -160, 192), gl], w)
            put(96, jnp.concatenate([s[0:32] + bias4(B_HEAD), s[32:160], s[160:] + bias4(B_TAIL)], axis=0))

        def qk_merged():
            kf = pltpu.bitcast(kb[rows_at(t1, -256, 96), gl], jnp.uint32)
            kd = pltpu.roll(pltpu.bitcast(kb[rows_at(t1, 32, 96), gl], jnp.uint32), 64, 1)
            ln = lax.broadcasted_iota(jnp.int32, kf.shape, 1) < 64
            la = pltpu.bitcast(jnp.where(ln, kf, kd), BF)
            lb = pltpu.bitcast(jnp.where(ln, kd, kf), BF)
            parts = []
            for k in range(3):
                w2a, w2b = b_w2(t1, g, k)
                rows = slice(32 * k, 32 * k + 32)
                parts.append(jnp.concatenate([_dot(la[rows], w2a), _dot(lb[rows], w2b)], axis=1))
            put(0, jnp.concatenate(parts, axis=0) + bias4(B_MRG))

        def qk_plain(ti):
            s = _dot(kb[_ds(t1 + ti - 2), gl], w)
            if ti == 2:
                s = s + bias4(B_DIAG)
            put(ti * 128 - 96, s)

        def prob(s_old):
            pr = jnp.exp2(s_old - m_cur)
            st['l'] = lfold(jnp.add, st['l'], pr)
            return pr

        def pv(ti, parts):
            for j in range(4):
                pj = jnp.concatenate([x[:, j * 128:(j + 1) * 128] for x in parts], axis=0).astype(BF)
                o = _dot(vtb[pl.ds(g * 128 + j * 32, 32), _ds(t2 + ti - 2)], pj)
                st['acc'][j] = o if st['acc'][j] is None else st['acc'][j] + o

        def fill():
            if filler is not None:
                filler()

        def far_parts(pms, pf):
            return [jnp.where(early[k], pms[k], 0.0) for k in range(3)] + [pf]

        def diag_parts(pms, pd):
            return [pd] + [jnp.where(early[k], 0.0, pms[k]) for k in range(3)]

        def split(pm):
            return [pm[32 * k:32 * k + 32] for k in range(3)]

        if nt2 == 3 and nt1 == 3:
            sm, sf, smid, sd = load(0, 96), load(96, 32), load(128, 128), load(256, 32)
            qk_wide()
            pm, pf = prob(sm), prob(sf)
            pms = split(pm)
            pv(0, far_parts(pms, pf))
            pv(1, [prob(smid)])
            qk_merged()
            pv(2, diag_parts(pms, prob(sd)))
        elif nt2 == 3:
            fill()
            sm, sf = load(0, 96), load(96, 32)
            pm, pf = prob(sm), prob(sf)
            pms = split(pm)
            pv(0, far_parts(pms, pf))
            fill()
            smid, sd = load(128, 128), load(256, 32)
            pv(1, [prob(smid)])
            fill()
            pv(2, diag_parts(pms, prob(sd)))
        else:
            for ti in range(3 - nt2, 3):
                pv(ti, [prob(load(ti * 128 - 96, 128))])
            if nt1 == 3:
                qk_merged()
                qk_wide()
            else:
                for ti in range(3 - nt1, 3):
                    qk_plain(ti)
        m_new = jnp.max(st['mx'], axis=0, keepdims=True) if nt1 else None
        return m_new, ((g, t2, st['acc'], st['l']) if nt2 else None)

    def ntiles(t):
        return min(t + 1, 3) if isinstance(t, int) else 3

    def acc_parts():
        a = acc_ref[...]
        return [a[:, j * 128:(j + 1) * 128] for j in range(4)]

    def b_body(t0, ms, do1=True, do2=True, fin_prev=True, filler=None):
        out = []
        prev = None
        if fin_prev:
            prev = (NG - 1, t0 - 1, acc_parts(), l_ref[...])
        for p in range(NBB):
            t2, t1 = t0 + p, t0 + p + NBB
            for g in range(NG):
                m, prev = b_unit(p, g, t2, ntiles(t2) if do2 else 0, ms[p * NG + g] if do2 else None,
                                 t1, ntiles(t1) if do1 else 0, prev, filler)
                out.append(m)
        if prev is not None:
            acc_ref[...] = jnp.concatenate(prev[2], axis=1)
            l_ref[...] = prev[3]
        return out

    ms = b_body(-NBB, None, do2=False, fin_prev=False)
    ms = b_body(0, ms, fin_prev=False)
    ms = lax.fori_loop(1, NQ // NBB - 1, lambda i, ms: tuple(b_body(i * NBB, list(ms))), tuple(ms))

    wob_cp.wait()
    ob_chunks = _offsets(OB_CH)
    outb_cps = out_copies(outb, ob_chunks, D, len(oa_chunks))
    fill = _Filler(oproj_pieces(ob, wob, outb, *ob_chunks[0]), NG * 3 * NBB)
    b_body(NQ - NBB, list(ms), do1=False, filler=fill)
    fill.finish()
    outb_cps[0].start()
    b_fin(NG - 1, NQ - 1, acc_parts(), l_ref[...])
    for c, (s0, n) in enumerate(ob_chunks):
        if c == 0:
            continue
        outb[pl.ds(s0, n), :] = _dot(ob[pl.ds(s0, n), :], wob[...]).astype(BF)
        outb_cps[c].start()
    for c in outa_cps + outb_cps:
        c.wait()


@jax.jit
def pallas_concat_heads__grouped_kv_mqa__sliding_block__prompt_kernel(
    A_x: jax.Array,
    A_wq: jax.Array,
    A_wk: jax.Array,
    A_wv: jax.Array,
    A_wo: jax.Array,
    B_x: jax.Array,
    B_wqkv: jax.Array,
    B_wo: jax.Array,
):
    any_spec = pl.BlockSpec(memory_space=pl.ANY)
    V = pltpu.VMEM
    scratch = [
        V((S, D), BF), V((D, D), BF), V((D, D), BF),
        V((S, D), BF), V((D, 3 * D), BF), V((D, D), BF),
        V((D + 2 * DH, D), BF), V((2 * D, D), BF),
        V((D, S), BF), V((S, 128), BF), V((DH, S), BF), V((S, D), BF),
        V((S, D), BF), V((D, S), BF),
        V((NB, S, 512), F32), V((NBB * NG, 288, 512), F32), V((288, 128), F32),
        V((DH, 512), F32), V((8, 512), F32),
        pltpu.SemaphoreType.DMA((S // XC,)), pltpu.SemaphoreType.DMA((10,)),
        pltpu.SemaphoreType.DMA((len(OA_CH) + len(OB_CH),)),
    ]
    out = pl.pallas_call(
        _kernel,
        out_shape=jax.ShapeDtypeStruct((S, 2 * D), BF),
        in_specs=[any_spec] * 8,
        out_specs=any_spec,
        scratch_shapes=scratch,
        compiler_params=pltpu.CompilerParams(vmem_limit_bytes=112 * 1024 * 1024),
    )(A_x.reshape(S, D), A_wq, A_wk.T, A_wv.T, A_wo, B_x.reshape(S, D), B_wqkv, B_wo)
    return out.reshape(1, S, 2 * D)
```
